```python
import os as _os
_os.environ.setdefault("JAX_PLATFORMS", "cpu")
import jax
import jax.numpy as jnp

def _softmax(x, axis=-1):
    return jax.nn.softmax(x, axis=axis)
def _gelu(x):
    return jax.nn.gelu(x, approximate=True)
def _silu(x):
    return jax.nn.silu(x)
def _sigmoid(x):
    return jax.nn.sigmoid(x)
def _layernorm(x, axis=-1, eps=1e-5):
    m = jnp.mean(x, axis=axis, keepdims=True)
    v = jnp.var(x, axis=axis, keepdims=True)
    return (x - m) / jnp.sqrt(v + eps)
def _scatter_add(tgt, idx, src, axis=0):
    return tgt.at[idx].add(src)
def _segment_sum(src, seg, n):
    return jax.ops.segment_sum(src, seg, n)
class _Rng:
    def __init__(self, key):
        self._k = key
    def _next(self):
        self._k, sub = jax.random.split(self._k)
        return sub
    def normal(self, shape):
        return jax.random.normal(self._next(), shape, dtype=jnp.bfloat16)
    def randint(self, lo, hi, shape):
        return jax.random.randint(self._next(), shape, lo, hi, dtype=jnp.int32)
    def uniform(self, shape, lo=0.0, hi=1.0):
        return jax.random.uniform(self._next(), shape, jnp.bfloat16, lo, hi)
    def permutation(self, n):
        return jax.random.permutation(self._next(), n)


kernel_name = 'concat_heads__mha_block__linear_attn_block__prompt'

def setup_inputs():
    _rng = _Rng(jax.random.key(int.from_bytes(__import__("os").urandom(4), "little")))
    _w = (lambda a: (lambda t: t.astype(jnp.bfloat16) if jnp.issubdtype(t.dtype, jnp.floating) else t)(jnp.asarray(a)))
    def _A_setup():
        B, S, D, H = 1, 2048, 1024, 32
        return {
            "x": _w((lambda *s: _rng.normal(s) * 0.2)(B, S, D)),
            "wqkv": _w((lambda *s: _rng.normal(s) * 0.2)(D, 3 * D)),
            "wo": _w((lambda *s: _rng.normal(s) * 0.05)(D, D)),
        }
    _A_in = _A_setup()

    def _B_setup():
        B, S, D = 1, 2048, 1024
        return {
            "x": _w((lambda *s: _rng.normal(s) * 0.05)(B, S, D)),
            "wqkv": _w((lambda *s: _rng.normal(s) * 1.6)(D, 3 * D)),
            "wo": _w((lambda *s: _rng.normal(s) * 0.1)(D, D)),
        }
    _B_in = _B_setup()

    return {
        "A_x": _A_in["x"],
        "A_wqkv": _A_in["wqkv"],
        "A_wo": _A_in["wo"],
        "B_x": _B_in["x"],
        "B_wqkv": _B_in["wqkv"],
        "B_wo": _B_in["wo"],
    }

def reference(A_x, A_wqkv, A_wo, B_x, B_wqkv, B_wo):
    def _A_ref(x, wqkv, wo):
        B, S, D = x.shape
        H = 32
        Dh = D // H
        qkv = (lambda x, *d: x.transpose(*d))((x @ wqkv).reshape(B, S, 3, H, Dh), 2, 0, 3, 1, 4)
        q, k, v = qkv[0], qkv[1], qkv[2]
        scores = jnp.einsum("bhqd,bhkd->bhqk", q, k) * (Dh ** -0.5)
        p = _softmax(scores, axis=-1)
        o = jnp.einsum("bhqk,bhkd->bhqd", p, v)
        return (lambda x, *d: x.transpose(*d))(o, 0, 2, 1, 3).reshape(B, S, D) @ wo

    def _B_ref(x, wqkv, wo):
        B, S, D = x.shape
        H = 32; Dh = D // H
        qkv = (lambda x, *d: x.transpose(*d))((x @ wqkv).reshape(B, S, 3, H, Dh), 2, 0, 3, 1, 4)
        q, k, v = qkv[0], qkv[1], qkv[2]
        phi = lambda t: jnp.where(t > 0, t + 1, jnp.exp(t)) + 1e-6
        pq, pk = phi(q), phi(k)
        kv = jnp.einsum("bhsd,bhse->bhde", pk, v)
        z = jnp.einsum("bhsd->bhd", pk)
        num = jnp.einsum("bhqd,bhde->bhqe", pq, kv)
        den = jnp.einsum("bhqd,bhd->bhq", pq, z)[..., None] + 1e-6
        o = num / den
        return (lambda x, *d: x.transpose(*d))(o, 0, 2, 1, 3).reshape(B, S, D) @ wo

    a = _A_ref(A_x, A_wqkv, A_wo)
    b = _B_ref(B_x, B_wqkv, B_wo)
    return jnp.concatenate([a, b], axis=-1)
```

```python
import functools
import math

import jax
import jax.numpy as jnp
import jax.experimental.pallas as pl
import jax.experimental.pallas.tpu as pltpu

S = 2048
D = 1024
H = 32
DH = 32
G = 8
LANES = 128

TQ = 512
CK = 128
NQ = S // TQ
NC = S // CK
NITEMS = H * NQ
UNROLL = 4
SKEW = 2
LAG = 2

WC = 256
NWC = 3 * D // WC
RM = 512
NR = S // RM
OM = 256
NO = S // OM

NT = (((1,), (1,)), ((), ()))
TN = (((0,), (0,)), ((), ()))
F32 = jnp.float32
BF16 = jnp.bfloat16
QSCALE = (DH ** -0.5) * math.log2(math.e)


def _bits(x):
    return jax.lax.bitcast_convert_type(x, jnp.int32)


def _unbits(x):
    return jax.lax.bitcast_convert_type(x, F32)


def _phi(t):
    return jnp.where(t > 0, t + 1.0, jnp.exp(t)) + 1e-6


def _kernel(xa_hbm, wa_hbm, woa_hbm, xb_hbm, wb_hbm, wob_hbm, out_hbm,
            xa, wa, woa, xb, wb, wob,
            qm, kk, vt, sa, sb, ot, zero_ref,
            pkt, vb, zrow, mm, ostage,
            in_sems, wa_sems, wb_sems, out_sems):
    def x_copy(src, dst, i, sem):
        return pltpu.make_async_copy(
            src.at[0, pl.ds(i * RM, RM), :], dst.at[pl.ds(i * RM, RM), :], sem)

    def w_copy(src, dst, j, sems):
        return pltpu.make_async_copy(
            src.at[:, pl.ds(j * WC, WC)], dst.at[j], sems.at[j])

    def full_copy(src, dst, sem):
        return pltpu.make_async_copy(src, dst, sem)

    def out_copy(slot, r, half):
        return pltpu.make_async_copy(
            ostage.at[slot],
            out_hbm.at[0, pl.ds(r * OM, OM), pl.ds(half * D, D)],
            out_sems.at[slot])

    x_copy(xa_hbm, xa, 0, in_sems.at[0]).start()
    w_copy(wa_hbm, wa, 0, wa_sems).start()
    for i in range(1, NR):
        x_copy(xa_hbm, xa, i, in_sems.at[i]).start()
    for j in range(1, NWC):
        w_copy(wa_hbm, wa, j, wa_sems).start()
    full_copy(xb_hbm.at[0], xb, in_sems.at[NR]).start()
    for j in range(NWC):
        w_copy(wb_hbm, wb, (j + 4) % NWC, wb_sems).start()
    full_copy(wob_hbm, wob, in_sems.at[NR + 1]).start()
    full_copy(woa_hbm, woa, in_sems.at[NR + 2]).start()

    zero_ref[...] = jnp.zeros_like(zero_ref)

    lane = jax.lax.broadcasted_iota(jnp.int32, (RM, LANES), 1)
    head_masks = [(lane >= DH * t) & (lane < DH * (t + 1)) for t in range(4)]
    GPC = WC // LANES

    for i in range(NR):
        x_copy(xa_hbm, xa, i, in_sems.at[i]).wait()

    def a_q_body(jj, carry):
        w_copy(wa_hbm, wa, jj, wa_sems).wait()
        for i in range(NR):
            rows = slice(i * RM, (i + 1) * RM)
            y = jnp.dot(xa[rows, :], wa[jj], preferred_element_type=F32) * QSCALE
            for gg in range(GPC):
                yg = y[:, gg * LANES:(gg + 1) * LANES]
                for t in range(4):
                    h = (jj * GPC + gg) * 4 + t
                    qm[h, rows, :] = jnp.where(head_masks[t], yg, 0.0).astype(BF16)
        return carry

    def a_k_body(jj, carry):
        j = jj + NWC // 3
        w_copy(wa_hbm, wa, j, wa_sems).wait()
        for i in range(NR):
            rows = slice(i * RM, (i + 1) * RM)
            y = jnp.dot(xa[rows, :], wa[j], preferred_element_type=F32).astype(BF16)
            for gg in range(GPC):
                kk[jj * GPC + gg, rows, :] = y[:, gg * LANES:(gg + 1) * LANES]
        return carry

    def a_v_body(jj, carry):
        j = jj + 2 * NWC // 3
        w_copy(wa_hbm, wa, j, wa_sems).wait()
        for i in range(NR):
            rows = slice(i * RM, (i + 1) * RM)
            y = jnp.dot(xa[rows, :], wa[j], preferred_element_type=F32)
            vt[pl.ds(pl.multiple_of(jj * WC, WC), WC), rows] = y.T.astype(BF16)
        return carry

    jax.lax.fori_loop(0, NWC // 3, a_q_body, 0)
    jax.lax.fori_loop(0, NWC // 3, a_k_body, 0)
    jax.lax.fori_loop(0, NWC // 3, a_v_body, 0)

    full_copy(xb_hbm.at[0], xb, in_sems.at[NR]).wait()

    def b_k_body(jj, carry):
        j = jj + NWC // 3
        w_copy(wb_hbm, wb, j, wb_sems).wait()
        zs = None
        for i in range(NR):
            rows = slice(i * RM, (i + 1) * RM)
            pk = _phi(jnp.dot(xb[rows, :], wb[j], preferred_element_type=F32))
            cs = jnp.sum(pk.reshape(RM // 8, 8, WC), axis=0)
            zs = cs if zs is None else zs + cs
            pkt[pl.ds(pl.multiple_of(jj * WC, WC), WC), rows] = pk.T.astype(BF16)
        zrow[jj] = jnp.broadcast_to(jnp.sum(zs, axis=0, keepdims=True), (8, WC))
        return carry

    def b_v_body(jj, carry):
        j = jj + 2 * NWC // 3
        w_copy(wb_hbm, wb, j, wb_sems).wait()
        for i in range(NR):
            rows = slice(i * RM, (i + 1) * RM)
            y = jnp.dot(xb[rows, :], wb[j], preferred_element_type=F32).astype(BF16)
            for gg in range(GPC):
                vb[jj * GPC + gg, rows, :] = y[:, gg * LANES:(gg + 1) * LANES]
        return carry

    jax.lax.fori_loop(0, NWC // 3, b_k_body, 0)
    jax.lax.fori_loop(0, NWC // 3, b_v_body, 0)

    full_copy(wob_hbm, wob, in_sems.at[NR + 1]).wait()
    r128 = jax.lax.broadcasted_iota(jnp.int32, (LANES, LANES), 0)
    c128 = jax.lax.broadcasted_iota(jnp.int32, (LANES, LANES), 1)
    same_head = (r128 // DH) == (c128 // DH)
    zts = []
    for g in range(G):
        gs = slice(g * LANES, (g + 1) * LANES)
        kv = jnp.dot(pkt[gs, :], vb[g], preferred_element_type=F32)
        kv = jnp.where(same_head, kv, 0.0).astype(BF16)
        mm[gs, :] = jnp.dot(kv, wob[gs, :], preferred_element_type=F32).astype(BF16)
    for j in range(NWC // 3):
        w_copy(wb_hbm, wb, j, wb_sems).wait()

    def b_out_body(r, carry):
        slot = r % 2
        rows = pl.ds(pl.multiple_of(r * OM, OM), OM)
        xr = xb[rows, :]
        parts = []
        for jj in range(NWC // 3):
            pq = _phi(jnp.dot(xr, wb[jj], preferred_element_type=F32))
            zr = zrow[jj]
            for gg in range(GPC):
                pqg = pq[:, gg * LANES:(gg + 1) * LANES]
                zg = zr[0:1, gg * LANES:(gg + 1) * LANES]
                zt = jnp.where(same_head, jnp.broadcast_to(zg, (LANES, LANES)), 0.0).astype(BF16)
                den = jax.lax.dot_general(pqg.astype(BF16), zt, NT,
                                          preferred_element_type=F32) + 1e-6
                parts.append((pqg / den).astype(BF16))
        a = jnp.concatenate(parts, axis=1)
        res = jnp.dot(a, mm[...], preferred_element_type=F32).astype(BF16)

        @pl.when(r >= 2)
        def _():
            out_copy(slot, r - 2, 1).wait()

        ostage[slot] = res
        out_copy(slot, r, 1).start()
        return carry

    jax.lax.fori_loop(0, NO, b_out_body, 0)
    out_copy(0, NO - 2, 1).wait()
    out_copy(1, NO - 1, 1).wait()

    bufs = (sa, sb)

    def item_coords(n):
        h = n % H
        off = pl.multiple_of((n // H) * TQ, TQ)
        return h, off

    def score_chunk(n, c, buf, mx):
        h, off = item_coords(n)
        s = jax.lax.dot_general(kk[h // 4, c * CK:(c + 1) * CK, :],
                                qm[h, pl.ds(off, TQ), :], NT,
                                preferred_element_type=F32)
        buf[c * CK:(c + 1) * CK, :] = s
        cm = jnp.max(s.reshape(CK // 8, 8, TQ), axis=0)
        return cm if mx is None else jnp.maximum(mx, cm)

    def finish_max(mx):
        return jnp.broadcast_to(jnp.max(mx, axis=0, keepdims=True), (8, TQ))

    mx = None
    for c in range(NC):
        mx = score_chunk(0, c, bufs[0], mx)
    m0 = finish_max(mx)
    mx = None
    for c in range(SKEW):
        mx = score_chunk(1, c, bufs[1], mx)
    mx0 = mx

    def attn_body(r, carry):
        m, mx = carry
        zero = zero_ref[...]
        n0 = r * UNROLL
        hist = []
        for u in range(UNROLL):
            n = n0 + u
            h, off = item_coords(n)
            hrow = pl.ds(pl.multiple_of(h * DH, DH), DH)
            buf = bufs[u % 2]
            acc = None
            l = None
            m_next = None
            for c in range(NC):
                cs = c + SKEW
                if cs < NC:
                    mx = score_chunk((n + 1) % NITEMS, cs, bufs[(u + 1) % 2], mx)
                    if cs == NC - 1:
                        m_next = finish_max(mx)
                        mx = None
                        dep = _bits(m_next)
                    else:
                        dep = _bits(mx)
                else:
                    mx = score_chunk((n + 2) % NITEMS, cs - NC, bufs[u % 2], mx)
                    dep = _bits(mx)
                mu = m
                if len(hist) >= LAG:
                    mu = _unbits(_bits(m) | (hist[-LAG] & zero))
                s = buf[c * CK:(c + 1) * CK, :].reshape(CK // 8, 8, TQ)
                p = jnp.exp2(s - mu[None])
                cl = jnp.sum(p, axis=0)
                l = cl if l is None else l + cl
                o = jnp.dot(vt[hrow, c * CK:(c + 1) * CK],
                            p.reshape(CK, TQ).astype(BF16),
                            preferred_element_type=F32)
                acc = o if acc is None else acc + o
                hist.append(dep ^ _bits(l))
            lt = jnp.sum(l, axis=0, keepdims=True)
            ot[hrow, pl.ds(off, TQ)] = (acc / lt).astype(BF16)
            m = m_next
        return m, mx

    jax.lax.fori_loop(0, NITEMS // UNROLL, attn_body, (m0, mx0))

    full_copy(woa_hbm, woa, in_sems.at[NR + 2]).wait()

    def a_out_body(r, carry):
        slot = r % 2
        cols = pl.ds(pl.multiple_of(r * OM, OM), OM)
        res = jax.lax.dot_general(ot[:, cols], woa[...], TN,
                                  preferred_element_type=F32).astype(BF16)

        @pl.when(r >= 2)
        def _():
            out_copy(slot, r - 2, 0).wait()

        ostage[slot] = res
        out_copy(slot, r, 0).start()
        return carry

    jax.lax.fori_loop(0, NO, a_out_body, 0)
    out_copy(0, NO - 2, 0).wait()
    out_copy(1, NO - 1, 0).wait()


@jax.jit
def pallas_concat_heads__mha_block__linear_attn_block__prompt_kernel(
    A_x: jax.Array,
    A_wqkv: jax.Array,
    A_wo: jax.Array,
    B_x: jax.Array,
    B_wqkv: jax.Array,
    B_wo: jax.Array,
):
    any_spec = pl.BlockSpec(memory_space=pl.ANY)
    scratch = [
        pltpu.VMEM((S, D), BF16),
        pltpu.VMEM((NWC, D, WC), BF16),
        pltpu.VMEM((D, D), BF16),
        pltpu.VMEM((S, D), BF16),
        pltpu.VMEM((NWC, D, WC), BF16),
        pltpu.VMEM((D, D), BF16),
        pltpu.VMEM((H, S, LANES), BF16),
        pltpu.VMEM((G, S, LANES), BF16),
        pltpu.VMEM((D, S), BF16),
        pltpu.VMEM((S, TQ), F32),
        pltpu.VMEM((S, TQ), F32),
        pltpu.VMEM((D, S), BF16),
        pltpu.VMEM((8, TQ), jnp.int32),
        pltpu.VMEM((D, S), BF16),
        pltpu.VMEM((G, S, LANES), BF16),
        pltpu.VMEM((NWC // 3, 8, WC), F32),
        pltpu.VMEM((D, D), BF16),
        pltpu.VMEM((2, OM, D), BF16),
        pltpu.SemaphoreType.DMA((NR + 3,)),
        pltpu.SemaphoreType.DMA((NWC,)),
        pltpu.SemaphoreType.DMA((NWC,)),
        pltpu.SemaphoreType.DMA((2,)),
    ]
    return pl.pallas_call(
        _kernel,
        out_shape=jax.ShapeDtypeStruct((1, S, 2 * D), BF16),
        in_specs=[any_spec] * 6,
        out_specs=any_spec,
        scratch_shapes=scratch,
        compiler_params=pltpu.CompilerParams(vmem_limit_bytes=110 * 1024 * 1024),
    )(A_x, A_wqkv, A_wo, B_x, B_wqkv, B_wo)
```

```python
import functools
import math

import jax
import jax.numpy as jnp
import jax.experimental.pallas as pl
import jax.experimental.pallas.tpu as pltpu

S = 2048
D = 1024
H = 32
DH = 32
G = 8
LANES = 128

TQ = 512
CK = 128
NQ = S // TQ
NC = S // CK
NITEMS = H * NQ
UNROLL = 8
SKEW = 1
LAG = 2
LAGL = 1

WC = 256
NWC = 3 * D // WC
NSEC = NWC // 3
GPC = WC // LANES
RM = 512
NR = S // RM
OM = 256
NO = S // OM
OUNROLL = 8
XPIECES = ((0, 128), (128, 128), (256, 256), (512, 512), (1024, 1024))

NT = (((1,), (1,)), ((), ()))
TN = (((0,), (0,)), ((), ()))
F32 = jnp.float32
BF16 = jnp.bfloat16
QSCALE = (DH ** -0.5) * math.log2(math.e)
scope = jax.named_scope


def _bits(x):
    return jax.lax.bitcast_convert_type(x, jnp.int32)


def _unbits(x):
    return jax.lax.bitcast_convert_type(x, F32)


def _pack(x):
    return pltpu.bitcast(x, jnp.uint32)


def _unpack(x):
    return pltpu.bitcast(x, BF16)


def _phi(t):
    return jnp.where(t > 0, t + 1.0, jnp.exp(t)) + 1e-6


def _kernel(xa_hbm, wa_hbm, woa_hbm, xb_hbm, wb_hbm, wob_hbm, out_hbm,
            xa, wa, xb, wb, wob,
            qm, kk, vt, sa, sb, zero_ref,
            pkb, lhst, wout, ostage,
            in_sems, wa_sems, wb_sems, out_sems):
    def xa_copy(i):
        r0, n = XPIECES[i]
        return pltpu.make_async_copy(
            xa_hbm.at[0, pl.ds(r0, n), :], xa.at[pl.ds(r0, n), :], in_sems.at[i])

    def wa_copy(j):
        return pltpu.make_async_copy(
            wa_hbm.at[:, pl.ds(j * WC, WC)], wa.at[j], wa_sems.at[j])

    def wb_copy(j):
        return pltpu.make_async_copy(
            wb_hbm.at[:, pl.ds(j * WC, WC)], wb.at[j], wb_sems.at[j])

    NX = len(XPIECES)
    xb_copy = pltpu.make_async_copy(xb_hbm.at[0], xb, in_sems.at[NX])
    wob_copy = pltpu.make_async_copy(wob_hbm, wob, in_sems.at[NX + 1])
    woa_copy = pltpu.make_async_copy(woa_hbm, wout.at[0], in_sems.at[NX + 2])

    def out_copy(half, r):
        return pltpu.make_async_copy(
            ostage.at[half, pl.ds(r * OM, OM), :],
            out_hbm.at[0, pl.ds(r * OM, OM), pl.ds(half * D, D)],
            out_sems.at[half * NO + r])

    QJ, KJ, VJ = 0, NSEC, 2 * NSEC

    xa_copy(0).start()
    wa_copy(VJ).start()
    xa_copy(1).start()
    wa_copy(QJ).start()

    zero_ref[...] = jnp.zeros_like(zero_ref)

    def a_q_tile(r0, n, jj):
        rows = pl.ds(r0, n)
        lane = jax.lax.broadcasted_iota(jnp.int32, (n // 2, LANES), 1)
        y = jnp.dot(xa[rows, :], wa[QJ + jj], preferred_element_type=F32) * QSCALE
        for gg in range(GPC):
            yg = _pack(y[:, gg * LANES:(gg + 1) * LANES].astype(BF16))
            for t in range(4):
                h = (jj * GPC + gg) * 4 + t
                keep = (lane >= DH * t) & (lane < DH * (t + 1))
                qm[h, pl.ds(r0 // 2, n // 2), :] = jnp.where(keep, yg, jnp.zeros_like(yg))

    def a_k_tile(r0, n, jj):
        rows = pl.ds(r0, n)
        y = jnp.dot(xa[rows, :], wa[KJ + jj], preferred_element_type=F32).astype(BF16)
        for gg in range(GPC):
            kk[jj * GPC + gg, pl.ds(r0 // 2, n // 2), :] = _pack(y[:, gg * LANES:(gg + 1) * LANES])

    def a_v_tile(r0, n, jj):
        rows = pl.ds(r0, n)
        y = jnp.dot(xa[rows, :], wa[VJ + jj], preferred_element_type=F32)
        vt[pl.ds(pl.multiple_of(jj * (WC // 2), WC // 2), WC // 2), rows] = _pack(y.T.astype(BF16))

    with scope('a_p0'):
        xa_copy(0).wait()
        wa_copy(VJ).wait()
        xa_copy(2).start()
        a_v_tile(0, 128, 0)
        xa_copy(1).wait()
        wa_copy(KJ).start()
        a_v_tile(128, 128, 0)
        wa_copy(QJ).wait()
        xa_copy(3).start()
        a_q_tile(0, 256, 0)
        xa_copy(2).wait()
        a_v_tile(256, 256, 0)
        a_q_tile(256, 256, 0)
        wa_copy(KJ).wait()
        xa_copy(4).start()
        a_k_tile(0, 512, 0)
        xa_copy(3).wait()
        a_v_tile(512, 512, 0)
        a_q_tile(512, 512, 0)
        a_k_tile(512, 512, 0)
        xa_copy(4).wait()
        for jj in range(1, NSEC):
            for j0 in (VJ, QJ, KJ):
                wa_copy(j0 + jj).start()
        for tile in (a_v_tile, a_q_tile, a_k_tile):
            for r0 in (1024, 1536):
                tile(r0, 512, 0)
        xb_copy.start()
        for jj in range(NSEC):
            for j0 in (KJ, QJ, VJ):
                wb_copy(j0 + jj).start()
        wob_copy.start()
        woa_copy.start()

    def a_p_body(jj, carry):
        for j0 in (VJ, QJ, KJ):
            wa_copy(j0 + jj).wait()
        for tile in (a_v_tile, a_q_tile, a_k_tile):
            for i in range(NR):
                tile(i * RM, RM, jj)
        return carry

    with scope('a_p'):
        jax.lax.fori_loop(1, NSEC, a_p_body, 0)

    xb_copy.wait()
    wob_copy.wait()
    r128 = jax.lax.broadcasted_iota(jnp.int32, (LANES, LANES), 0)
    c128 = jax.lax.broadcasted_iota(jnp.int32, (LANES, LANES), 1)
    same_head = (r128 // DH) == (c128 // DH)

    def b_p_body(jj, carry):
        for j0 in (KJ, QJ, VJ):
            wb_copy(j0 + jj).wait()
        drows = pl.ds(pl.multiple_of(jj * WC, WC), WC)
        zs = None
        for i in range(NR):
            rows = slice(i * RM, (i + 1) * RM)
            pk = _phi(jnp.dot(xb[rows, :], wb[KJ + jj], preferred_element_type=F32))
            cs = jnp.sum(pk.reshape(RM // 8, 8, WC), axis=0)
            zs = cs if zs is None else zs + cs
            pkb[rows, :] = pk.astype(BF16)
        zc = jnp.broadcast_to(jnp.sum(zs, axis=0, keepdims=True), (LANES, WC)).T
        zc = zc.reshape(WC // DH, DH, LANES)
        for i in range(NR):
            rows = slice(i * RM, (i + 1) * RM)
            pq = _phi(jnp.dot(xb[rows, :], wb[QJ + jj], preferred_element_type=F32)).T
            for t in range(RM // LANES):
                pt = pq[:, t * LANES:(t + 1) * LANES].reshape(WC // DH, DH, LANES)
                den = jnp.sum(pt * zc, axis=1, keepdims=True) + 1e-6
                lhst[1, drows, i * RM + t * LANES:i * RM + (t + 1) * LANES] = (
                    (pt / den).reshape(WC, LANES).astype(BF16))
        txt = jnp.concatenate(
            [jax.lax.dot_general(xb[:, t * RM:(t + 1) * RM], pkb[...], TN,
                                 preferred_element_type=F32).astype(BF16)
             for t in range(D // RM)], axis=0)
        kvs = []
        for gg in range(GPC):
            gs = slice(gg * LANES, (gg + 1) * LANES)
            kv = jax.lax.dot_general(txt[:, gs], wb[VJ + jj, :, gs], TN,
                                     preferred_element_type=F32)
            kvs.append(jnp.where(same_head, kv, 0.0).astype(BF16))
        for gg in range(GPC):
            grows = pl.ds(pl.multiple_of(jj * WC + gg * LANES, LANES), LANES)
            wout[1, grows, :] = jnp.dot(kvs[gg], wob[grows, :],
                                        preferred_element_type=F32).astype(BF16)
        return carry

    with scope('b_p'):
        jax.lax.fori_loop(0, NSEC, b_p_body, 0)

    bufs = (sa, sb)

    def item_coords(n):
        h = n % H
        off = pl.multiple_of((n // H) * TQ, TQ)
        return h, off

    def score_chunk(n, c, buf, mx):
        h, off = item_coords(n)
        off2 = pl.multiple_of((n // H) * (TQ // 2), TQ // 2)
        s = jax.lax.dot_general(_unpack(kk[h // 4, c * CK // 2:(c + 1) * CK // 2, :]),
                                _unpack(qm[h, pl.ds(off2, TQ // 2), :]), NT,
                                preferred_element_type=F32)
        buf[c * CK:(c + 1) * CK, :] = s
        cm = jnp.max(s.reshape(CK // 8, 8, TQ), axis=0)
        return cm if mx is None else jnp.maximum(mx, cm)

    def finish_max(mx):
        return jnp.broadcast_to(jnp.max(mx, axis=0, keepdims=True), (8, TQ))

    with scope('kv_prol'):
        mx = None
        for c in range(NC):
            mx = score_chunk(0, c, bufs[0], mx)
        m0 = finish_max(mx)
        mx = None
        for c in range(SKEW):
            mx = score_chunk(1, c, bufs[1], mx)
        mx0 = mx

    def attn_body(r, carry):
        m, mx = carry
        zero = zero_ref[...]
        n0 = r * UNROLL
        hist = []
        histl = []
        for u in range(UNROLL):
            n = n0 + u
            h, off = item_coords(n)
            hrow = pl.ds(pl.multiple_of(h * DH, DH), DH)
            hrow2 = pl.ds(pl.multiple_of(h * (DH // 2), DH // 2), DH // 2)
            buf = bufs[u % 2]
            acc = None
            l = None
            m_next = None
            for c in range(NC):
                cs = c + SKEW
                if cs < NC:
                    mx = score_chunk((n + 1) % NITEMS, cs, bufs[(u + 1) % 2], mx)
                    if cs == NC - 1:
                        m_next = finish_max(mx)
                        mx = None
                        dep = _bits(m_next)
                    else:
                        dep = _bits(mx)
                else:
                    mx = score_chunk((n + 2) % NITEMS, cs - NC, bufs[u % 2], mx)
                    dep = _bits(mx)
                mu = m
                d = None
                if len(hist) >= LAG:
                    d = hist[-LAG]
                if len(histl) >= LAGL:
                    d = histl[-LAGL] if d is None else d ^ histl[-LAGL]
                if d is not None:
                    mu = _unbits(_bits(m) | (d & zero))
                s = buf[c * CK:(c + 1) * CK, :].reshape(CK // 8, 8, TQ)
                p = jnp.exp2(s - mu[None])
                for t in range(CK // 16 - 1, -1, -1):
                    cl = p[2 * t + 1] + p[2 * t]
                    l = cl if l is None else l + cl
                o = jnp.dot(_unpack(vt[hrow2, c * CK:(c + 1) * CK]),
                            p.reshape(CK, TQ).astype(BF16),
                            preferred_element_type=F32)
                acc = o if acc is None else o + acc
                hist.append(dep)
                histl.append(_bits(l))
            lt = jnp.sum(l, axis=0, keepdims=True)
            lhst[0, hrow, pl.ds(off, TQ)] = (acc / lt).astype(BF16)
            m = m_next
        return m, mx

    with scope('attn'):
        jax.lax.fori_loop(0, NITEMS // UNROLL, attn_body, (m0, mx0))

    woa_copy.wait()

    def out_body(rr, carry):
        for u in range(OUNROLL):
            t = rr * OUNROLL + u
            half = 1 - t // NO
            r = t % NO
            rows = pl.ds(pl.multiple_of(r * OM, OM), OM)
            ostage[half, rows, :] = jax.lax.dot_general(
                lhst[half, :, rows], wout[half], TN,
                preferred_element_type=F32).astype(BF16)
            out_copy(half, r).start()
        return carry

    with scope('out'):
        jax.lax.fori_loop(0, 2 * NO // OUNROLL, out_body, 0)
    with scope('owait'):
        for half in (1, 0):
            for r in range(NO):
                out_copy(half, r).wait()


@jax.jit
def pallas_concat_heads__mha_block__linear_attn_block__prompt_kernel(
    A_x: jax.Array,
    A_wqkv: jax.Array,
    A_wo: jax.Array,
    B_x: jax.Array,
    B_wqkv: jax.Array,
    B_wo: jax.Array,
):
    any_spec = pl.BlockSpec(memory_space=pl.ANY)
    scratch = [
        pltpu.VMEM((S, D), BF16),
        pltpu.VMEM((NWC, D, WC), BF16),
        pltpu.VMEM((S, D), BF16),
        pltpu.VMEM((NWC, D, WC), BF16),
        pltpu.VMEM((D, D), BF16),
        pltpu.VMEM((H, S // 2, LANES), jnp.uint32),
        pltpu.VMEM((G, S // 2, LANES), jnp.uint32),
        pltpu.VMEM((D // 2, S), jnp.uint32),
        pltpu.VMEM((S, TQ), F32),
        pltpu.VMEM((S, TQ), F32),
        pltpu.VMEM((8, TQ), jnp.int32),
        pltpu.VMEM((S, WC), BF16),
        pltpu.VMEM((2, D, S), BF16),
        pltpu.VMEM((2, D, D), BF16),
        pltpu.VMEM((2, S, D), BF16),
        pltpu.SemaphoreType.DMA((len(XPIECES) + 3,)),
        pltpu.SemaphoreType.DMA((NWC,)),
        pltpu.SemaphoreType.DMA((NWC,)),
        pltpu.SemaphoreType.DMA((2 * NO,)),
    ]
    return pl.pallas_call(
        _kernel,
        out_shape=jax.ShapeDtypeStruct((1, S, 2 * D), BF16),
        in_specs=[any_spec] * 6,
        out_specs=any_spec,
        scratch_shapes=scratch,
        compiler_params=pltpu.CompilerParams(vmem_limit_bytes=110 * 1024 * 1024),
    )(A_x, A_wqkv, A_wo, B_x, B_wqkv, B_wo)
```

```python
import math

import jax
import jax.numpy as jnp
import jax.experimental.pallas as pl
import jax.experimental.pallas.tpu as pltpu

S = 2048
D = 1024
H = 32
DH = 32
G = 8
LANES = 128

TQ = 512
CK = 128
NQ = S // TQ
NC = S // CK
NITEMS = H * NQ
UNROLL = 16
SKEW = 1
LAG = 2
LAGL = 1

WC = 256
NWC = 3 * D // WC
NSEC = NWC // 3
GPC = WC // LANES
RM = 512
NR = S // RM
QJ, KJ, VJ = 0, NSEC, 2 * NSEC

XPIECES = ((0, 128), (128, 128), (256, 256), (512, 512), (1024, 1024))
OPIECES = tuple((r, 256) for r in range(0, 1792, 256)) + ((1792, 128), (1920, 128))
NX = len(XPIECES)
NO = len(OPIECES)

NT = (((1,), (1,)), ((), ()))
TN = (((0,), (0,)), ((), ()))
F32 = jnp.float32
BF16 = jnp.bfloat16
U32 = jnp.uint32
QSCALE = (DH ** -0.5) * math.log2(math.e)


def _mo(x, m):
    return x if isinstance(x, int) else pl.multiple_of(x, m)


def _bits(x):
    return jax.lax.bitcast_convert_type(x, jnp.int32)


def _unbits(x):
    return jax.lax.bitcast_convert_type(x, F32)


def _pack(x):
    return pltpu.bitcast(x, U32)


def _unpack(x):
    return pltpu.bitcast(x, BF16)


def _phi(t):
    return jnp.where(t > 0, t + 1.0, jnp.exp(t)) + 1e-6


def _kernel(xa_hbm, wa_hbm, woa_hbm, xb_hbm, wb_hbm, wob_hbm, out_hbm,
            xa, wa, xb, wb, wob,
            qm, kk, vt, sa, sb, zero_ref,
            pkb, lhst, wout, ostage,
            in_sems, wa_sems, wb_sems, out_sems):
    def xa_copy(i):
        r0, n = XPIECES[i]
        return pltpu.make_async_copy(
            xa_hbm.at[0, pl.ds(r0, n), :], xa.at[pl.ds(r0, n), :], in_sems.at[i])

    def wa_copy(j):
        return pltpu.make_async_copy(
            wa_hbm.at[:, pl.ds(j * WC, WC)], wa.at[j], wa_sems.at[j])

    def wb_copy(j):
        return pltpu.make_async_copy(
            wb_hbm.at[:, pl.ds(j * WC, WC)], wb.at[j], wb_sems.at[j])

    xb_copy = pltpu.make_async_copy(xb_hbm.at[0], xb, in_sems.at[NX])
    wob_copy = pltpu.make_async_copy(wob_hbm, wob, in_sems.at[NX + 1])
    woa_copy = pltpu.make_async_copy(woa_hbm, wout.at[0], in_sems.at[NX + 2])

    def out_copy(half, k):
        r0, n = OPIECES[k]
        return pltpu.make_async_copy(
            ostage.at[half, pl.ds(r0, n), :],
            out_hbm.at[0, pl.ds(r0, n), pl.ds(half * D, D)],
            out_sems.at[half * NO + k])

    xa_copy(0).start()
    wa_copy(VJ).start()
    xa_copy(1).start()
    wa_copy(QJ).start()

    zero_ref[...] = jnp.zeros_like(zero_ref)

    def zfill(c, carry):
        sb[pl.ds(pl.multiple_of(c * CK, CK), CK), :] = jnp.zeros((CK, TQ), F32)
        return carry

    jax.lax.fori_loop(0, NC, zfill, 0)

    def a_q_tile(r0, n, jj):
        lane = jax.lax.broadcasted_iota(jnp.int32, (n // 2, LANES), 1)
        y = jnp.dot(xa[pl.ds(r0, n), :], wa[QJ + jj], preferred_element_type=F32) * QSCALE
        for gg in range(GPC):
            yg = _pack(y[:, gg * LANES:(gg + 1) * LANES].astype(BF16))
            for t in range(4):
                h = (jj * GPC + gg) * 4 + t
                keep = (lane >= DH * t) & (lane < DH * (t + 1))
                qm[h, pl.ds(r0 // 2, n // 2), :] = jnp.where(keep, yg, jnp.zeros_like(yg))

    def a_k_tile(r0, n, jj):
        y = jnp.dot(xa[pl.ds(r0, n), :], wa[KJ + jj],
                    preferred_element_type=F32).astype(BF16)
        for gg in range(GPC):
            kk[jj * GPC + gg, pl.ds(r0 // 2, n // 2), :] = _pack(
                y[:, gg * LANES:(gg + 1) * LANES])

    def a_v_tile(r0, n, jj):
        y = jnp.dot(xa[pl.ds(r0, n), :], wa[VJ + jj], preferred_element_type=F32)
        vt[pl.ds(_mo(jj * (WC // 2), WC // 2), WC // 2), pl.ds(r0, n)] = _pack(
            y.T.astype(BF16))

    xa_copy(0).wait()
    wa_copy(VJ).wait()
    xa_copy(2).start()
    a_v_tile(0, 128, 0)
    xa_copy(1).wait()
    wa_copy(KJ).start()
    a_v_tile(128, 128, 0)
    wa_copy(QJ).wait()
    xa_copy(3).start()
    a_q_tile(0, 256, 0)
    xa_copy(2).wait()
    a_v_tile(256, 256, 0)
    a_q_tile(256, 256, 0)
    wa_copy(KJ).wait()
    xa_copy(4).start()
    a_k_tile(0, 512, 0)
    xa_copy(3).wait()
    a_v_tile(512, 512, 0)
    a_q_tile(512, 512, 0)
    a_k_tile(512, 512, 0)
    xa_copy(4).wait()
    for jj in range(1, NSEC):
        for j0 in (VJ, QJ, KJ):
            wa_copy(j0 + jj).start()
    for tile in (a_v_tile, a_q_tile, a_k_tile):
        for r0 in (1024, 1536):
            tile(r0, 512, 0)
    xb_copy.start()
    for jj in range(NSEC):
        for j0 in (KJ, QJ, VJ):
            wb_copy(j0 + jj).start()
    wob_copy.start()
    woa_copy.start()

    def a_p_body(jj, carry):
        for j0 in (VJ, QJ, KJ):
            wa_copy(j0 + jj).wait()
        for tile in (a_v_tile, a_q_tile, a_k_tile):
            for i in range(NR):
                tile(i * RM, RM, jj)
        return carry

    jax.lax.fori_loop(1, NSEC, a_p_body, 0)

    xb_copy.wait()
    wob_copy.wait()
    r128 = jax.lax.broadcasted_iota(jnp.int32, (LANES, LANES), 0)
    c128 = jax.lax.broadcasted_iota(jnp.int32, (LANES, LANES), 1)
    same_head = (r128 // DH) == (c128 // DH)

    def b_p_body(jj, carry):
        for j0 in (KJ, QJ, VJ):
            wb_copy(j0 + jj).wait()
        drows = pl.ds(_mo(jj * WC, WC), WC)
        zs = None
        for i in range(NR):
            rows = slice(i * RM, (i + 1) * RM)
            pk = _phi(jnp.dot(xb[rows, :], wb[KJ + jj], preferred_element_type=F32))
            cs = jnp.sum(pk.reshape(RM // 8, 8, WC), axis=0)
            zs = cs if zs is None else zs + cs
            pkb[i * RM // 2:(i + 1) * RM // 2, :] = _pack(pk.astype(BF16))
        zc = jnp.broadcast_to(jnp.sum(zs, axis=0, keepdims=True), (LANES, WC)).T
        zc = zc.reshape(WC // DH, DH, LANES)
        for i in range(NR):
            rows = slice(i * RM, (i + 1) * RM)
            pq = _phi(jnp.dot(xb[rows, :], wb[QJ + jj], preferred_element_type=F32)).T
            for t in range(RM // LANES):
                pt = pq[:, t * LANES:(t + 1) * LANES].reshape(WC // DH, DH, LANES)
                den = jnp.sum(pt * zc, axis=1, keepdims=True) + 1e-6
                lhst[1, drows, i * RM + t * LANES:i * RM + (t + 1) * LANES] = (
                    (pt / den).reshape(WC, LANES).astype(BF16))
        txt = jnp.concatenate(
            [jax.lax.dot_general(xb[:, t * RM:(t + 1) * RM], _unpack(pkb[...]), TN,
                                 preferred_element_type=F32).astype(BF16)
             for t in range(D // RM)], axis=0)
        kvs = []
        for gg in range(GPC):
            gs = slice(gg * LANES, (gg + 1) * LANES)
            kv = jax.lax.dot_general(txt[:, gs], wb[VJ + jj, :, gs], TN,
                                     preferred_element_type=F32)
            kvs.append(jnp.where(same_head, kv, 0.0).astype(BF16))
        for gg in range(GPC):
            grows = pl.ds(_mo(jj * WC + gg * LANES, LANES), LANES)
            wout[1, grows, :] = jnp.dot(kvs[gg], wob[grows, :],
                                        preferred_element_type=F32).astype(BF16)
        return carry

    jax.lax.fori_loop(0, NSEC, b_p_body, 0)

    bufs = (sa, sb)

    def item_coords(n):
        return n % H, n // H

    def score_chunk(n, c, buf, mx):
        h, j = item_coords(n)
        s = jax.lax.dot_general(
            _unpack(kk[h // 4, c * CK // 2:(c + 1) * CK // 2, :]),
            _unpack(qm[h, pl.ds(_mo(j * (TQ // 2), TQ // 2), TQ // 2), :]), NT,
            preferred_element_type=F32)
        buf[c * CK:(c + 1) * CK, :] = s
        cm = jnp.max(s.reshape(CK // 8, 8, TQ), axis=0)
        return cm if mx is None else jnp.maximum(mx, cm)

    def finish_max(mx):
        return jnp.broadcast_to(jnp.max(mx, axis=0, keepdims=True), (8, TQ))

    def pv_chunk(n, c, buf, mu, acc, l):
        h, _ = item_coords(n)
        s = buf[c * CK:(c + 1) * CK, :].reshape(CK // 8, 8, TQ)
        p = jnp.exp2(s - mu[None])
        for t in range(CK // 16 - 1, -1, -1):
            cl = p[2 * t + 1] + p[2 * t]
            l = cl if l is None else l + cl
        o = jnp.dot(
            _unpack(vt[pl.ds(_mo(h * (DH // 2), DH // 2), DH // 2), c * CK:(c + 1) * CK]),
            p.reshape(CK, TQ).astype(BF16), preferred_element_type=F32)
        acc = o if acc is None else o + acc
        return acc, l

    def pv_finish(n, acc, l):
        h, j = item_coords(n)
        lt = jnp.sum(l, axis=0, keepdims=True)
        lhst[0, pl.ds(_mo(h * DH, DH), DH), pl.ds(_mo(j * TQ, TQ), TQ)] = (
            (acc / lt).astype(BF16))

    def hinted(m, d, zero):
        return _unbits(_bits(m) | (d & zero))

    woa_copy.wait()
    mx0 = None
    for c in range(SKEW):
        mx0 = score_chunk(0, c, bufs[0], mx0)
    m0 = jnp.zeros((8, TQ), F32)

    def attn_body(r, carry):
        m, mx = carry
        zero = zero_ref[...]
        n0 = r * UNROLL + (NITEMS - 1)
        hist = []
        histl = []
        for u in range(UNROLL):
            n = (n0 + u) % NITEMS
            buf = bufs[(u + 1) % 2]
            acc = None
            l = None
            m_next = None
            for c in range(NC):
                cs = c + SKEW
                if cs < NC:
                    mx = score_chunk((n0 + u + 1) % NITEMS, cs, bufs[u % 2], mx)
                    if cs == NC - 1:
                        m_next = finish_max(mx)
                        mx = None
                        dep = _bits(m_next)
                    else:
                        dep = _bits(mx)
                else:
                    mx = score_chunk((n0 + u + 2) % NITEMS, cs - NC, buf, mx)
                    dep = _bits(mx)
                d = None
                if len(hist) >= LAG:
                    d = hist[-LAG]
                if len(histl) >= LAGL:
                    d = histl[-LAGL] if d is None else d ^ histl[-LAGL]
                mu = m if d is None else hinted(m, d, zero)
                acc, l = pv_chunk(n, c, buf, mu, acc, l)
                hist.append(dep)
                histl.append(_bits(l))
            pv_finish(n, acc, l)
            m = m_next
        return m, mx

    m_last, _ = jax.lax.fori_loop(0, NITEMS // UNROLL, attn_body, (m0, mx0))

    zero = zero_ref[...]
    acc = None
    l = None
    npc = D // LANES
    for c in range(NC):
        mu = m_last if l is None else hinted(m_last, _bits(l), zero)
        acc, l = pv_chunk(NITEMS - 1, c, bufs[1], mu, acc, l)
        k, t = c // npc, c % npc
        r0, n = OPIECES[k]
        if t == 0:
            lhs = lhst[1, :, pl.ds(r0, n)].T
        cols = slice(t * LANES, (t + 1) * LANES)
        ostage[1, pl.ds(r0, n), cols] = jnp.dot(
            lhs, wout[1, :, cols], preferred_element_type=F32).astype(BF16)
        if t == npc - 1:
            out_copy(1, k).start()
    pv_finish(NITEMS - 1, acc, l)
    for half in (1, 0):
        for k, (r0, n) in enumerate(OPIECES):
            if half == 1 and k < NC // npc:
                continue
            rows = pl.ds(r0, n)
            ostage[half, rows, :] = jax.lax.dot_general(
                lhst[half, :, rows], wout[half], TN,
                preferred_element_type=F32).astype(BF16)
            out_copy(half, k).start()
    for half in (1, 0):
        for k in range(NO):
            out_copy(half, k).wait()


@jax.jit
def pallas_concat_heads__mha_block__linear_attn_block__prompt_kernel(
    A_x: jax.Array,
    A_wqkv: jax.Array,
    A_wo: jax.Array,
    B_x: jax.Array,
    B_wqkv: jax.Array,
    B_wo: jax.Array,
):
    any_spec = pl.BlockSpec(memory_space=pl.ANY)
    scratch = [
        pltpu.VMEM((S, D), BF16),
        pltpu.VMEM((NWC, D, WC), BF16),
        pltpu.VMEM((S, D), BF16),
        pltpu.VMEM((NWC, D, WC), BF16),
        pltpu.VMEM((D, D), BF16),
        pltpu.VMEM((H, S // 2, LANES), U32),
        pltpu.VMEM((G, S // 2, LANES), U32),
        pltpu.VMEM((D // 2, S), U32),
        pltpu.VMEM((S, TQ), F32),
        pltpu.VMEM((S, TQ), F32),
        pltpu.VMEM((8, TQ), jnp.int32),
        pltpu.VMEM((S // 2, WC), U32),
        pltpu.VMEM((2, D, S), BF16),
        pltpu.VMEM((2, D, D), BF16),
        pltpu.VMEM((2, S, D), BF16),
        pltpu.SemaphoreType.DMA((NX + 3,)),
        pltpu.SemaphoreType.DMA((NWC,)),
        pltpu.SemaphoreType.DMA((NWC,)),
        pltpu.SemaphoreType.DMA((2 * NO,)),
    ]
    return pl.pallas_call(
        _kernel,
        out_shape=jax.ShapeDtypeStruct((1, S, 2 * D), BF16),
        in_specs=[any_spec] * 6,
        out_specs=any_spec,
        scratch_shapes=scratch,
        compiler_params=pltpu.CompilerParams(vmem_limit_bytes=110 * 1024 * 1024),
    )(A_x, A_wqkv, A_wo, B_x, B_wqkv, B_wo)
```

```python
import math

import jax
import jax.numpy as jnp
import jax.experimental.pallas as pl
import jax.experimental.pallas.tpu as pltpu

S = 2048
D = 1024
H = 32
DH = 32
G = 8
LANES = 128

TQ = 512
CK = 128
NQ = S // TQ
NC = S // CK
NITEMS = H * NQ
UNROLL = 16
SKEW = 1
LAG = 2
LAGL = 1
SPLIT = (5, 3)

WC = 256
NWC = 3 * D // WC
NSEC = NWC // 3
GPC = WC // LANES
RM = 512
NR = S // RM
QJ, KJ, VJ = 0, NSEC, 2 * NSEC

STAGES = (
    (0, 1024, 0, 128, True),
    (1024, 1024, 0, 128, False),
    (0, S, 128, 128, True),
    (0, S, 256, 256, True),
    (0, S, 512, 512, True),
)
NSTART = 3
ISSUE = {0: 3, 2: 4}

OPIECES = tuple((r, 256) for r in range(0, 2048, 256))
LS = 8
NO = len(OPIECES)

NT = (((1,), (1,)), ((), ()))
TN = (((0,), (0,)), ((), ()))
F32 = jnp.float32
BF16 = jnp.bfloat16
U32 = jnp.uint32
QSCALE = (DH ** -0.5) * math.log2(math.e)


def _mo(x, m):
    return x if isinstance(x, int) else pl.multiple_of(x, m)


def _bits(x):
    return jax.lax.bitcast_convert_type(x, jnp.int32)


def _unbits(x):
    return jax.lax.bitcast_convert_type(x, F32)


def _pack(x):
    return pltpu.bitcast(x, U32)


def _unpack(x):
    return pltpu.bitcast(x, BF16)


def _phi(t):
    return jnp.where(t > 0, t + 1.0, jnp.exp(t)) + 1e-6


def _kernel(xa_hbm, wa_hbm, woa_hbm, xb_hbm, wb_hbm, wob_hbm, out_hbm,
            xa, wa, xb, wb, wob,
            qm, kk, vt, sa, sb, zero_ref,
            pkb, lhst, wout, ostage, yacc,
            sems):
    def stage_copies(si):
        r0, n, k0, kn, with_w = STAGES[si]
        cps = [pltpu.make_async_copy(
            xa_hbm.at[0, pl.ds(r0, n), pl.ds(k0, kn)],
            xa.at[pl.ds(r0, n), pl.ds(k0, kn)], sems.at[si])]
        if with_w:
            cps += [pltpu.make_async_copy(
                wa_hbm.at[pl.ds(k0, kn), pl.ds(j * WC, WC)],
                wa.at[j, pl.ds(k0, kn), :], sems.at[si]) for j in (VJ, QJ, KJ)]
        return cps

    def wa_copy(j0, jj):
        j = j0 + jj
        return pltpu.make_async_copy(
            wa_hbm.at[:, pl.ds(j * WC, WC)], wa.at[j], sems.at[jj])

    BSEM = 0
    OSEM = NSEC
    b_copies = [pltpu.make_async_copy(xb_hbm.at[0], xb, sems.at[BSEM])]
    b_copies += [
        pltpu.make_async_copy(wb_hbm.at[:, pl.ds(j * WC, WC)], wb.at[j], sems.at[BSEM])
        for j in range(NWC)]
    b_copies += [pltpu.make_async_copy(wob_hbm, wob, sems.at[BSEM]),
                 pltpu.make_async_copy(woa_hbm, wout.at[0], sems.at[BSEM])]

    def out_copy(half, k, c0=0, nc=D):
        r0, n = OPIECES[k]
        return pltpu.make_async_copy(
            ostage.at[half, pl.ds(r0, n), pl.ds(c0, nc)],
            out_hbm.at[0, pl.ds(r0, n), pl.ds(half * D + c0, nc)],
            sems.at[OSEM])

    for si in range(NSTART):
        for cp in stage_copies(si):
            cp.start()

    zero_ref[...] = jnp.zeros_like(zero_ref)

    def zfill(c, carry):
        sb[pl.ds(pl.multiple_of(c * CK, CK), CK), :] = jnp.zeros((CK, TQ), F32)
        return carry

    jax.lax.fori_loop(0, NC, zfill, 0)

    def a_dot(j, r0, n, k0=0, kn=D):
        return jnp.dot(xa[pl.ds(r0, n), pl.ds(k0, kn)], wa[j, pl.ds(k0, kn), :],
                       preferred_element_type=F32)

    def a_q_out(y, r0, n, jj):
        lane = jax.lax.broadcasted_iota(jnp.int32, (n // 2, LANES), 1)
        y = y * QSCALE
        for gg in range(GPC):
            yg = _pack(y[:, gg * LANES:(gg + 1) * LANES].astype(BF16))
            for t in range(4):
                h = (jj * GPC + gg) * 4 + t
                keep = (lane >= DH * t) & (lane < DH * (t + 1))
                qm[h, pl.ds(r0 // 2, n // 2), :] = jnp.where(keep, yg, jnp.zeros_like(yg))

    def a_k_out(y, r0, n, jj):
        y = y.astype(BF16)
        for gg in range(GPC):
            kk[jj * GPC + gg, pl.ds(r0 // 2, n // 2), :] = _pack(
                y[:, gg * LANES:(gg + 1) * LANES])

    def a_v_out(y, r0, n, jj):
        vt[pl.ds(_mo(jj * (WC // 2), WC // 2), WC // 2), pl.ds(r0, n)] = _pack(
            y.T.astype(BF16))

    secs = ((VJ, a_v_out), (QJ, a_q_out), (KJ, a_k_out))

    for si, (r0, n, k0, kn, _) in enumerate(STAGES):
        for cp in stage_copies(si):
            cp.wait()
        if si in ISSUE:
            for cp in stage_copies(ISSUE[si]):
                cp.start()
        if si == len(STAGES) - 1:
            for jj in range(1, NSEC):
                for j0 in (VJ, QJ, KJ):
                    wa_copy(j0, jj).start()
        for ai, (j0, out) in enumerate(secs):
            for rr in range(r0, r0 + n, RM):
                y = a_dot(j0, rr, RM, k0, kn)
                if k0 > 0:
                    y = y + yacc[ai, pl.ds(rr, RM), :]
                if k0 + kn < D:
                    yacc[ai, pl.ds(rr, RM), :] = y
                else:
                    out(y, rr, RM, 0)
    for cp in b_copies:
        cp.start()

    def a_p_body(jj, carry):
        for j0 in (VJ, QJ, KJ):
            wa_copy(j0, jj).wait()
        for j0, out in secs:
            for i in range(NR):
                out(a_dot(j0 + jj, i * RM, RM), i * RM, RM, jj)
        return carry

    jax.lax.fori_loop(1, NSEC, a_p_body, 0)

    for cp in b_copies:
        cp.wait()
    r128 = jax.lax.broadcasted_iota(jnp.int32, (LANES, LANES), 0)
    c128 = jax.lax.broadcasted_iota(jnp.int32, (LANES, LANES), 1)
    same_head = (r128 // DH) == (c128 // DH)

    def b_p_body(jj, carry):
        drows = pl.ds(_mo(jj * WC, WC), WC)
        zs = None
        for i in range(NR):
            rows = slice(i * RM, (i + 1) * RM)
            pk = _phi(jnp.dot(xb[rows, :], wb[KJ + jj], preferred_element_type=F32))
            cs = jnp.sum(pk.reshape(RM // 8, 8, WC), axis=0)
            zs = cs if zs is None else zs + cs
            pkb[i * RM // 2:(i + 1) * RM // 2, :] = _pack(pk.astype(BF16))
        zc = jnp.broadcast_to(jnp.sum(zs, axis=0, keepdims=True), (LANES, WC)).T
        zc = zc.reshape(WC // DH, DH, LANES)
        for i in range(NR):
            rows = slice(i * RM, (i + 1) * RM)
            pq = _phi(jnp.dot(xb[rows, :], wb[QJ + jj], preferred_element_type=F32)).T
            for t in range(RM // LANES):
                pt = pq[:, t * LANES:(t + 1) * LANES].reshape(WC // DH, DH, LANES)
                den = jnp.sum(pt * zc, axis=1, keepdims=True) + 1e-6
                lhst[1, drows, i * RM + t * LANES:i * RM + (t + 1) * LANES] = (
                    (pt / den).reshape(WC, LANES).astype(BF16))
        txt = jnp.concatenate(
            [jax.lax.dot_general(xb[:, t * RM:(t + 1) * RM], _unpack(pkb[...]), TN,
                                 preferred_element_type=F32).astype(BF16)
             for t in range(D // RM)], axis=0)
        kvs = []
        for gg in range(GPC):
            gs = slice(gg * LANES, (gg + 1) * LANES)
            kv = jax.lax.dot_general(txt[:, gs], wb[VJ + jj, :, gs], TN,
                                     preferred_element_type=F32)
            kvs.append(jnp.where(same_head, kv, 0.0).astype(BF16))
        for gg in range(GPC):
            grows = pl.ds(_mo(jj * WC + gg * LANES, LANES), LANES)
            wout[1, grows, :] = jnp.dot(kvs[gg], wob[grows, :],
                                        preferred_element_type=F32).astype(BF16)
        return carry

    jax.lax.fori_loop(0, NSEC, b_p_body, 0)

    bufs = (sa, sb)

    def item_coords(n):
        return n & (H - 1), n >> 5

    def score_chunk(n, c, buf, mx):
        h, j = item_coords(n)
        s = jax.lax.dot_general(
            _unpack(kk[h >> 2, c * CK // 2:(c + 1) * CK // 2, :]),
            _unpack(qm[h, pl.ds(_mo(j * (TQ // 2), TQ // 2), TQ // 2), :]), NT,
            preferred_element_type=F32)
        buf[c * CK:(c + 1) * CK, :] = s
        cm = jnp.max(s.reshape(CK // 8, 8, TQ), axis=0)
        return cm if mx is None else jnp.maximum(mx, cm)

    def finish_max(mx):
        return jnp.broadcast_to(jnp.max(mx, axis=0, keepdims=True), (8, TQ))

    def hinted(m, d, zero):
        return _unbits(_bits(m) | (d & zero))

    def pv_chunk(n, c, buf, mu, acc, l):
        h, _ = item_coords(n)
        s = buf[c * CK:(c + 1) * CK, :].reshape(CK // 8, 8, TQ)
        parts = []
        hi = CK // 8
        for npair in SPLIT:
            lo = hi - 2 * npair
            if parts:
                mu = hinted(mu, _bits(l), zero_ref[...])
            pb = jnp.exp2(s[lo:hi] - mu[None])
            for t in range(npair - 1, -1, -1):
                cl = pb[2 * t + 1] + pb[2 * t]
                l = cl if l is None else l + cl
            parts.insert(0, pb)
            hi = lo
        p = jnp.concatenate(parts, axis=0)
        o = jnp.dot(
            _unpack(vt[pl.ds(_mo(h * (DH // 2), DH // 2), DH // 2), c * CK:(c + 1) * CK]),
            p.reshape(CK, TQ).astype(BF16), preferred_element_type=F32)
        acc = o if acc is None else o + acc
        return acc, l

    def pv_finish(n, acc, l):
        h, j = item_coords(n)
        lt = jnp.sum(l, axis=0, keepdims=True)
        lhst[0, pl.ds(_mo(h * DH, DH), DH), pl.ds(_mo(j * TQ, TQ), TQ)] = (
            (acc / lt).astype(BF16))

    mx0 = None
    for c in range(SKEW):
        mx0 = score_chunk(0, c, bufs[0], mx0)
    m0 = jnp.zeros((8, TQ), F32)

    def attn_body(r, carry):
        m, mx = carry
        zero = zero_ref[...]
        n0 = r * UNROLL + (NITEMS - 1)
        hist = []
        histl = []
        for u in range(UNROLL):
            n = (n0 + u) & (NITEMS - 1)
            buf = bufs[(u + 1) % 2]
            acc = None
            l = None
            m_next = None
            for c in range(NC):
                cs = c + SKEW
                if cs < NC:
                    mx = score_chunk((n0 + u + 1) & (NITEMS - 1), cs, bufs[u % 2], mx)
                    if cs == NC - 1:
                        m_next = finish_max(mx)
                        mx = None
                        dep = _bits(m_next)
                    else:
                        dep = _bits(mx)
                else:
                    mx = score_chunk((n0 + u + 2) & (NITEMS - 1), cs - NC, buf, mx)
                    dep = _bits(mx)
                d = None
                if len(hist) >= LAG:
                    d = hist[-LAG]
                if len(histl) >= LAGL:
                    d = histl[-LAGL] if d is None else d ^ histl[-LAGL]
                mu = m if d is None else hinted(m, d, zero)
                acc, l = pv_chunk(n, c, buf, mu, acc, l)
                hist.append(dep)
                histl.append(_bits(l))
            pv_finish(n, acc, l)
            m = m_next
        return m, mx

    m_last, _ = jax.lax.fori_loop(0, NITEMS // UNROLL, attn_body, (m0, mx0))

    zero = zero_ref[...]
    acc = None
    l = None
    npc = D // LANES
    for c in range(NC):
        mu = m_last if l is None else hinted(m_last, _bits(l), zero)
        acc, l = pv_chunk(NITEMS - 1, c, bufs[1], mu, acc, l)
        k, t = c // npc, c % npc
        r0, n = OPIECES[k]
        if t == 0:
            lhs = lhst[1, :, pl.ds(r0, n)].T
        cols = slice(t * LANES, (t + 1) * LANES)
        ostage[1, pl.ds(r0, n), cols] = jnp.dot(
            lhs, wout[1, :, cols], preferred_element_type=F32).astype(BF16)
        if t == npc - 1:
            out_copy(1, k).start()
    pv_finish(NITEMS - 1, acc, l)
    started = [out_copy(1, k) for k in range(NC // npc)]
    for half in (1, 0):
        for k, (r0, n) in enumerate(OPIECES):
            if half == 1 and k < NC // npc:
                continue
            rows = pl.ds(r0, n)
            nsplit = LS if (half == 0 and k == NO - 1) else 1
            w = D // nsplit
            for t in range(nsplit):
                cols = pl.ds(t * w, w)
                ostage[half, rows, cols] = jax.lax.dot_general(
                    lhst[half, :, rows], wout[half, :, cols], TN,
                    preferred_element_type=F32).astype(BF16)
                cp = out_copy(half, k, t * w, w)
                cp.start()
                started.append(cp)
    for cp in started:
        cp.wait()


@jax.jit
def pallas_concat_heads__mha_block__linear_attn_block__prompt_kernel(
    A_x: jax.Array,
    A_wqkv: jax.Array,
    A_wo: jax.Array,
    B_x: jax.Array,
    B_wqkv: jax.Array,
    B_wo: jax.Array,
):
    any_spec = pl.BlockSpec(memory_space=pl.ANY)
    scratch = [
        pltpu.VMEM((S, D), BF16),
        pltpu.VMEM((NWC, D, WC), BF16),
        pltpu.VMEM((S, D), BF16),
        pltpu.VMEM((NWC, D, WC), BF16),
        pltpu.VMEM((D, D), BF16),
        pltpu.VMEM((H, S // 2, LANES), U32),
        pltpu.VMEM((G, S // 2, LANES), U32),
        pltpu.VMEM((D // 2, S), U32),
        pltpu.VMEM((S, TQ), F32),
        pltpu.VMEM((S, TQ), F32),
        pltpu.VMEM((8, TQ), jnp.int32),
        pltpu.VMEM((S // 2, WC), U32),
        pltpu.VMEM((2, D, S), BF16),
        pltpu.VMEM((2, D, D), BF16),
        pltpu.VMEM((2, S, D), BF16),
        pltpu.VMEM((3, S, WC), F32),
        pltpu.SemaphoreType.DMA((max(len(STAGES), NSEC + 1),)),
    ]
    return pl.pallas_call(
        _kernel,
        out_shape=jax.ShapeDtypeStruct((1, S, 2 * D), BF16),
        in_specs=[any_spec] * 6,
        out_specs=any_spec,
        scratch_shapes=scratch,
        compiler_params=pltpu.CompilerParams(vmem_limit_bytes=110 * 1024 * 1024),
    )(A_x, A_wqkv, A_wo, B_x, B_wqkv, B_wo)
```
